```python
import os as _os
_os.environ.setdefault("JAX_PLATFORMS", "cpu")
import jax
import jax.numpy as jnp

def _softmax(x, axis=-1):
    return jax.nn.softmax(x, axis=axis)
def _gelu(x):
    return jax.nn.gelu(x, approximate=True)
def _silu(x):
    return jax.nn.silu(x)
def _sigmoid(x):
    return jax.nn.sigmoid(x)
def _layernorm(x, axis=-1, eps=1e-5):
    m = jnp.mean(x, axis=axis, keepdims=True)
    v = jnp.var(x, axis=axis, keepdims=True)
    return (x - m) / jnp.sqrt(v + eps)
def _scatter_add(tgt, idx, src, axis=0):
    return tgt.at[idx].add(src)
def _segment_sum(src, seg, n):
    return jax.ops.segment_sum(src, seg, n)
class _Rng:
    def __init__(self, key):
        self._k = key
    def _next(self):
        self._k, sub = jax.random.split(self._k)
        return sub
    def normal(self, shape):
        return jax.random.normal(self._next(), shape, dtype=jnp.bfloat16)
    def randint(self, lo, hi, shape):
        return jax.random.randint(self._next(), shape, lo, hi, dtype=jnp.int32)
    def uniform(self, shape, lo=0.0, hi=1.0):
        return jax.random.uniform(self._next(), shape, jnp.bfloat16, lo, hi)
    def permutation(self, n):
        return jax.random.permutation(self._next(), n)


kernel_name = 'concat_heads__gqa_block_cached__gqa_block_cached__near_ridge'

def setup_inputs():
    _rng = _Rng(jax.random.key(int.from_bytes(__import__("os").urandom(4), "little")))
    _w = (lambda a: (lambda t: t.astype(jnp.bfloat16) if jnp.issubdtype(t.dtype, jnp.floating) else t)(jnp.asarray(a)))
    def _A_setup():
        B, Sq, D = 8, 240, 640
        Hq, Hkv, Sk, Dh = 32, 32, 1024, 192
        assert Hq % Hkv == 0, (Hq, Hkv)
        return {
            "x": _w((lambda *s: _rng.normal(s) * 0.8)(B, Sq, D)),
            "k_cache": _w((lambda *s: _rng.normal(s) * 0.8)(B, Hkv, Sk, Dh)),
            "v_cache": _w((lambda *s: _rng.normal(s) * 0.05)(B, Hkv, Sk, Dh)),
            "wq": _w((lambda *s: _rng.normal(s) * 0.8)(D, Hq * Dh) * (D ** -0.5)),
            "wo": _w((lambda *s: _rng.normal(s) * 0.05)(Hq * Dh, D) * ((Hq * Dh) ** -0.5)),
        }
    _A_in = _A_setup()

    def _B_setup():
        B, Sq, D = 8, 240, 640
        Hq, Hkv, Sk, Dh = 32, 32, 1024, 192
        assert Hq % Hkv == 0, (Hq, Hkv)
        return {
            "x": _w((lambda *s: _rng.normal(s) * 0.8)(B, Sq, D)),
            "k_cache": _w((lambda *s: _rng.normal(s) * 0.8)(B, Hkv, Sk, Dh)),
            "v_cache": _w((lambda *s: _rng.normal(s) * 0.05)(B, Hkv, Sk, Dh)),
            "wq": _w((lambda *s: _rng.normal(s) * 0.8)(D, Hq * Dh) * (D ** -0.5)),
            "wo": _w((lambda *s: _rng.normal(s) * 0.05)(Hq * Dh, D) * ((Hq * Dh) ** -0.5)),
        }
    _B_in = _B_setup()

    return {
        "A_x": _A_in["x"],
        "A_k_cache": _A_in["k_cache"],
        "A_v_cache": _A_in["v_cache"],
        "A_wq": _A_in["wq"],
        "A_wo": _A_in["wo"],
        "B_x": _B_in["x"],
        "B_k_cache": _B_in["k_cache"],
        "B_v_cache": _B_in["v_cache"],
        "B_wq": _B_in["wq"],
        "B_wo": _B_in["wo"],
    }

def reference(A_x, A_k_cache, A_v_cache, A_wq, A_wo, B_x, B_k_cache, B_v_cache, B_wq, B_wo):
    def _A_ref(x, k_cache, v_cache, wq, wo):
        B, Sq, D = x.shape
        Hq, Dh = 32, 192
        Hkv = k_cache.shape[1]
        rep = Hq // Hkv
        q = (lambda x, *d: x.transpose(*d))((x @ wq).reshape(B, Sq, Hq, Dh), 0, 2, 1, 3)
        k = jnp.repeat(k_cache, rep, axis=1)
        v = jnp.repeat(v_cache, rep, axis=1)
        scores = jnp.einsum("bhqd,bhkd->bhqk", q, k) * (Dh ** -0.5)
        p = _softmax(scores, axis=-1)
        o = jnp.einsum("bhqk,bhkd->bhqd", p, v)
        return (lambda x, *d: x.transpose(*d))(o, 0, 2, 1, 3).reshape(B, Sq, Hq * Dh) @ wo

    def _B_ref(x, k_cache, v_cache, wq, wo):
        B, Sq, D = x.shape
        Hq, Dh = 32, 192
        Hkv = k_cache.shape[1]
        rep = Hq // Hkv
        q = (lambda x, *d: x.transpose(*d))((x @ wq).reshape(B, Sq, Hq, Dh), 0, 2, 1, 3)
        k = jnp.repeat(k_cache, rep, axis=1)
        v = jnp.repeat(v_cache, rep, axis=1)
        scores = jnp.einsum("bhqd,bhkd->bhqk", q, k) * (Dh ** -0.5)
        p = _softmax(scores, axis=-1)
        o = jnp.einsum("bhqk,bhkd->bhqd", p, v)
        return (lambda x, *d: x.transpose(*d))(o, 0, 2, 1, 3).reshape(B, Sq, Hq * Dh) @ wo

    a = _A_ref(A_x, A_k_cache, A_v_cache, A_wq, A_wo)
    b = _B_ref(B_x, B_k_cache, B_v_cache, B_wq, B_wo)
    return jnp.concatenate([a, b], axis=-1)
```

```python
import jax
import jax.numpy as jnp
import numpy as np
from jax.experimental import pallas as pl
from jax.experimental.pallas import tpu as pltpu

_SCALE = float(192 ** -0.5 * np.log2(np.e))
_NT = (((1,), (1,)), ((), ()))
_NP = 2


def _qproj(x_ref, wq_ref, j):
    q = jnp.dot(x_ref[...], wq_ref[:, j * 384:(j + 1) * 384], preferred_element_type=jnp.float32) * _SCALE
    q = q.astype(jnp.bfloat16)
    t0, t1, t2 = q[:, 0:128], q[:, 128:256], q[:, 256:384]
    lane = jax.lax.broadcasted_iota(jnp.int32, (240, 128), 1)
    zero = jnp.zeros_like(t1)
    q0 = jnp.concatenate([t0, jnp.where(lane < 64, t1, zero)], axis=1)
    q1 = jnp.concatenate([jnp.where(lane >= 64, t1, zero), t2], axis=1)
    return q0, q1


def _qk(q, kt_ref, j, h):
    base = j * 384 + h * 128
    return jnp.dot(q, kt_ref[base:base + 256, :], preferred_element_type=jnp.float32)


def _sm(s):
    m = jnp.max(s, axis=1, keepdims=True)
    p = jnp.exp2(s - m)
    l = jnp.sum(p, axis=1, keepdims=True)
    return p.astype(jnp.bfloat16), l


def _pv(p, vt_ref, j, h):
    base = j * 384 + h * 192
    return jax.lax.dot_general(vt_ref[base:base + 192, :], p, _NT, preferred_element_type=jnp.float32)


def _oproj(ot0, ot1, l0, l1, wo_ref, j):
    o = jnp.concatenate([ot0, ot1], axis=0).T
    i0 = 1.0 / l0
    i1 = 1.0 / l1
    lane = jax.lax.broadcasted_iota(jnp.int32, (240, 128), 1)
    mid = jnp.where(lane < 64, i0, i1)
    o = jnp.concatenate([o[:, 0:128] * i0, o[:, 128:256] * mid, o[:, 256:384] * i1], axis=1).astype(jnp.bfloat16)
    return jnp.dot(o, wo_ref[j * 384:(j + 1) * 384, :], preferred_element_type=jnp.float32)


def _kernel(xa, ka, va, wqa, woa, xb, kb, vb, wqb, wob, out_ref, acc_ref):
    hg = pl.program_id(0)
    b = pl.program_id(1)
    nhg = pl.num_programs(0)

    @pl.when(hg == 0)
    def _():
        acc_ref[b] = jnp.zeros((240, 1280), jnp.float32)

    for j in range(_NP):
        qa0, qa1 = _qproj(xa, wqa, j)
        qb0, qb1 = _qproj(xb, wqb, j)
        sa0 = _qk(qa0, ka, j, 0)
        sa1 = _qk(qa1, ka, j, 1)
        pa0, la0 = _sm(sa0)
        ota0 = _pv(pa0, va, j, 0)
        sb0 = _qk(qb0, kb, j, 0)
        pa1, la1 = _sm(sa1)
        ota1 = _pv(pa1, va, j, 1)
        sb1 = _qk(qb1, kb, j, 1)
        pb0, lb0 = _sm(sb0)
        otb0 = _pv(pb0, vb, j, 0)
        pb1, lb1 = _sm(sb1)
        otb1 = _pv(pb1, vb, j, 1)
        ra = _oproj(ota0, ota1, la0, la1, woa, j)
        acc_ref[b, :, 0:640] += ra
        rb = _oproj(otb0, otb1, lb0, lb1, wob, j)
        acc_ref[b, :, 640:1280] += rb

    @pl.when(hg == nhg - 1)
    def _():
        out_ref[b] = acc_ref[b].astype(jnp.bfloat16)


@jax.jit
def pallas_concat_heads__gqa_block_cached__gqa_block_cached__near_ridge_kernel(
    A_x, A_k_cache, A_v_cache, A_wq, A_wo, B_x, B_k_cache, B_v_cache, B_wq, B_wo,
):
    W = _NP * 384

    def kv(a):
        return jnp.swapaxes(a, 2, 3).reshape(8, 32 * 192, 1024)

    xs = pl.BlockSpec((None, 240, 640), lambda hg, b: (b, 0, 0))
    ks = pl.BlockSpec((None, W, 1024), lambda hg, b: (b, hg, 0))
    wqs = pl.BlockSpec((640, W), lambda hg, b: (0, hg))
    wos = pl.BlockSpec((W, 640), lambda hg, b: (hg, 0))
    return pl.pallas_call(
        _kernel,
        grid=(16 // _NP, 8),
        in_specs=[xs, ks, ks, wqs, wos] * 2,
        out_specs=pl.BlockSpec((8, 240, 1280), lambda i, j: (0, 0, 0)),
        out_shape=jax.ShapeDtypeStruct((8, 240, 1280), jnp.bfloat16),
        scratch_shapes=[pltpu.VMEM((8, 240, 1280), jnp.float32)],
        compiler_params=pltpu.CompilerParams(
            dimension_semantics=("arbitrary", "arbitrary"),
            vmem_limit_bytes=100 * 1024 * 1024,
        ),
        name="gqa2",
    )(A_x, kv(A_k_cache), kv(A_v_cache), A_wq, A_wo, B_x, kv(B_k_cache), kv(B_v_cache), B_wq, B_wo)
```

```python
import contextlib
import jax
import jax.numpy as jnp
import numpy as np
from jax.experimental import pallas as pl
from jax.experimental.pallas import tpu as pltpu

SCALE = float(192**-0.5 * np.log2(np.e))
NT = (((1,),(1,)),((),()))
f32 = jnp.float32; bf16 = jnp.bfloat16

def qproj(x, wq):
    q = jnp.dot(x, wq, preferred_element_type=f32) * SCALE
    q = q.astype(bf16)
    t0, t1, t2 = q[:, 0:128], q[:, 128:256], q[:, 256:384]
    lane = jax.lax.broadcasted_iota(jnp.int32, (240,128), 1)
    zero = jnp.zeros_like(t1)
    q0 = jnp.concatenate([t0, jnp.where(lane < 64, t1, zero)], axis=1)
    q1 = jnp.concatenate([jnp.where(lane >= 64, t1, zero), t2], axis=1)
    return q0, q1
def qk(q, kt_ref, h):
    base = h*128
    return jnp.dot(q, kt_ref[base:base+256, :], preferred_element_type=f32)
def sm(s):
    m = jnp.max(s, axis=1, keepdims=True)
    p = jnp.exp2(s - m)
    l = jnp.sum(p, axis=1, keepdims=True)
    return p.astype(bf16), l
def pv(p, vt_ref, h):
    base = h*192
    return jax.lax.dot_general(vt_ref[base:base+192, :], p, NT, preferred_element_type=f32)
def rcp(l):
    r = pl.reciprocal(l, approx=True)
    return r * (2.0 - l * r)
def oproj(ot0, ot1, l0, l1, wo):
    o = jnp.concatenate([ot0, ot1], axis=0).T
    i0 = rcp(l0); i1 = rcp(l1)
    lane = jax.lax.broadcasted_iota(jnp.int32, (240,128), 1)
    mid = jnp.where(lane < 64, i0, i1)
    o = jnp.concatenate([o[:, 0:128]*i0, o[:,128:256]*mid, o[:,256:384]*i1], axis=1).astype(bf16)
    return jnp.dot(o, wo, preferred_element_type=f32)

def pair_a(xa, xb, wqa, wqb, ka, va, kb, vb, woa, wob, acc, stage=None):
    qa0, qa1 = qproj(xa[...], wqa[...])
    qb0, qb1 = qproj(xb[...], wqb[...])
    sa0 = qk(qa0, ka, 0)
    sa1 = qk(qa1, ka, 1)
    pa0, la0 = sm(sa0)
    ota0 = pv(pa0, va, 0)
    sb0 = qk(qb0, kb, 0)
    pa1, la1 = sm(sa1)
    ota1 = pv(pa1, va, 1)
    sb1 = qk(qb1, kb, 1)
    pb0, lb0 = sm(sb0)
    otb0 = pv(pb0, vb, 0)
    pb1, lb1 = sm(sb1)
    otb1 = pv(pb1, vb, 1)
    ra = oproj(ota0, ota1, la0, la1, woa[...])
    na = acc[:, 0:640] + ra
    acc[:, 0:640] = na
    if stage is not None: stage[:, 0:640] = na.astype(bf16)
    rb = oproj(otb0, otb1, lb0, lb1, wob[...])
    nb = acc[:, 640:1280] + rb
    acc[:, 640:1280] = nb
    if stage is not None: stage[:, 640:1280] = nb.astype(bf16)


def order_a(NP):
    ops = []
    for j in range(NP):
        ua, ub = 2*j, 2*j+1
        a0,a1,b0,b1 = 2*ua, 2*ua+1, 2*ub, 2*ub+1
        ops += [('qp',ua),('qp',ub),('qk',a0),('qk',a1),('sm',a0),('pv',a0),('qk',b0),('sm',a1),('pv',a1),('qk',b1),('sm',b0),('pv',b0),('sm',b1),('pv',b1),('op',ua),('op',ub)]
    return ops

def order_rot(NP, variant=0):
    NU = 2*NP; NH = 2*NU
    ops = [('qp',0),('qp',1),('qk',0)]
    for h in range(NH):
        slot = []
        qk = [('qk',h+1)] if h+1 < NH else []
        smm = [('sm',h)]
        pvv = [('pv',h-1)] if h >= 1 else []
        pr = []
        if h % 2 == 0:
            u = h//2 + 1
            if h >= 2 and u < NU: pr = [('qp',u)]
        else:
            u = (h-1)//2 - 1
            if u >= 0 and h < NH-1: pr = [('op',u)]
        if variant == 0: slot = qk + smm + pvv + pr
        elif variant == 1: slot = smm + qk + pvv + pr
        elif variant == 2: slot = pvv + qk + smm + pr
        elif variant == 3: slot = smm + pvv + qk + pr
        elif variant == 4: slot = pr + qk + smm + pvv
        elif variant == 5: slot = qk + pvv + smm + pr
        elif variant == 6: slot = pvv + smm + qk + pr
        elif variant == 7: slot = smm + pr + qk + pvv
        ops += slot
    ops += [('pv',NH-1),('op',NU-2),('op',NU-1)]
    return ops

def run_ops(ops, xs, wqs, ks, vs, wos, acc, stage):
    st = {}
    for op, i in ops:
        if op == 'qp':
            s, j = i % 2, i // 2
            q0, q1 = qproj(xs[s][...], wqs(s, j)[...])
            st['q', 2*i] = q0; st['q', 2*i+1] = q1
        elif op == 'qk':
            u = i // 2; s, j = u % 2, u // 2
            st['s', i] = qk(st.pop(('q', i)), ks(s, j), i % 2)
        elif op == 'sm':
            st['p', i], st['l', i] = sm(st.pop(('s', i)))
        elif op == 'pv':
            u = i // 2; s, j = u % 2, u // 2
            st['o', i] = pv(st.pop(('p', i)), vs(s, j), i % 2)
        elif op == 'op':
            s, j = i % 2, i // 2
            r = oproj(st.pop(('o', 2*i)), st.pop(('o', 2*i+1)), st.pop(('l', 2*i)), st.pop(('l', 2*i+1)), wos(s, j)[...])
            c = slice(640*s, 640*s+640)
            n = acc[:, c] + r
            acc[:, c] = n
            if stage is not None:
                stage[:, c] = n.astype(bf16)
    assert not st, st.keys()


def make(NP=4, vmem=110*1024*1024, flags=None, nobc=True, scopes=False, order='a', variant=0, explore=False, SS=2):
    NSC = (lambda n: jax.named_scope(n)) if scopes else (lambda n: contextlib.nullcontext())
    NHG = 16//NP
    NS = 8*NHG
    def kernel(xa_h, ka_h, va_h, wqa_h, woa_h, xb_h, kb_h, vb_h, wqb_h, wob_h, out_h,
               xbuf, kv, wq, wo, acc, stage, s_kv, s_x, s_w, s_out):
        kvh = [ka_h, kb_h, va_h, vb_h]
        xh = [xa_h, xb_h]
        wqh = [wqa_h, wqb_h]; woh = [woa_h, wob_h]
        cp = pltpu.make_async_copy
        def x_start(b, slot):
            for s in range(2): cp(xh[s].at[b], xbuf.at[slot, s], s_x.at[slot]).start()
        def x_wait(slot):
            cp(xbuf.at[slot], xbuf.at[slot], s_x.at[slot]).wait()
        def kvp_start(b, p, slot, j):
            for i in range(4): cp(kvh[i].at[b, p], kv.at[slot, j, i], s_kv.at[slot, j]).start()
        def kvp_wait(slot, j):
            cp(kv.at[slot, j], kv.at[slot, j], s_kv.at[slot, j]).wait()
        def kvs_start(b, hg, slot):
            for i in range(4): cp(kvh[i].at[b, pl.ds(hg*NP, NP)], kv.at[slot, :, i], s_kv.at[slot, 0]).start()
        def kvs_wait(slot):
            cp(kv.at[slot], kv.at[slot], s_kv.at[slot, 0]).wait()
        def wp_start(p, wslot, j, sj):
            for s in range(2):
                cp(wqh[s].at[:, pl.ds(pl.multiple_of(p*384, 384), 384)], wq.at[wslot, j, s], s_w.at[sj]).start()
            for s in range(2):
                cp(woh[s].at[pl.ds(pl.multiple_of(p*384, 384), 384), :], wo.at[wslot, j, s], s_w.at[sj]).start()
        def wp_wait(wslot, j):
            cp(wq.at[wslot, j], wq.at[wslot, j], s_w.at[j]).wait()
            cp(wo.at[wslot, j], wo.at[wslot, j], s_w.at[j]).wait()
        def ws_start(hg):
            for j in range(NP): wp_start(hg*NP + j, hg & 1, j, 0)
        def ws_wait(wslot):
            cp(wq.at[wslot], wq.at[wslot], s_w.at[0]).wait()
            cp(wo.at[wslot], wo.at[wslot], s_w.at[0]).wait()
        def out_cp(b):
            return cp(stage.at[b], out_h.at[b], s_out.at[b])

        def run(ops, slot, wslot, b, js):
            run_ops(ops, [xbuf.at[slot, 0], xbuf.at[slot, 1]],
                      lambda s, j: wq.at[wslot, js(j), s], lambda s, j: kv.at[slot, js(j), s],
                      lambda s, j: kv.at[slot, js(j), 2+s], lambda s, j: wo.at[wslot, js(j), s],
                      acc.at[b], stage.at[b])

        with NSC("prologue"):
            x_start(0, 0)
            wp_start(0, 0, 0, 0)
            kvp_start(0, 0, 0, 0)
            acc[...] = jnp.zeros(acc.shape, f32)
        NSI = SS*NP
        def s_iter(i, _):
            ts = i // NP if NP > 1 else i
            j = i % NP if NP > 1 else 0
            i1 = i + 1
            ts1 = i1 // NP if NP > 1 else i1
            j1 = i1 % NP if NP > 1 else 0
            with NSC("s_issue"):
                @pl.when(i1 < NSI)
                def _():
                    @pl.when(j1 == 0)
                    def _():
                        x_start(ts1, ts1 & 1)
                    kvp_start(ts1, j1, ts1 & 1, j1)
                    @pl.when(i1 < NP)
                    def _():
                        wp_start(j1, 0, j1, j1)
                @pl.when(i >= NSI - NP)
                def _():
                    k = i - (NSI - NP)
                    kvp_start(SS % 8, (SS // 8)*NP + k, SS & 1, k)
                    @pl.when(k == 0)
                    def _():
                        x_start(SS % 8, SS & 1)
            with NSC("s_wait"):
                @pl.when(j == 0)
                def _():
                    x_wait(ts & 1)
                @pl.when(i < NP)
                def _():
                    wp_wait(0, j)
                kvp_wait(ts & 1, j)
            with NSC("s_body"):
                run(order_a(1), ts & 1, 0, ts, lambda _: j)
            return 0
        if not explore:
            jax.lax.fori_loop(0, NSI, s_iter, 0)
            with NSC("s_exit"):
                kvs_start((SS+1) % 8, (SS+1)//8, (SS+1) & 1)
                x_start((SS+1) % 8, (SS+1) & 1)
                for j in range(NP): kvp_wait(SS & 1, j)
                x_wait(SS & 1)

        def step(t, _):
            b = t & 7; hg = t >> 3; slot = t & 1; wslot = hg & 1
            with NSC("m_body"):
                ops = order_a(NP) if order == 'a' else order_rot(NP, variant)
                run(ops, slot, wslot, b, lambda j: j)
            with NSC("m_dma"):
                t2 = t + 2
                @pl.when(t2 < NS)
                def _():
                    kvs_start(t2 & 7, t2 >> 3, slot)
                    x_start(t2 & 7, slot)
                @pl.when(hg == NHG-1)
                def _():
                    out_cp(b).start()
                if NHG > 1:
                    @pl.when(jnp.logical_and(b == 4, hg + 1 < NHG))
                    def _():
                        ws_start(hg+1)
                    @pl.when(jnp.logical_and(b == 7, hg + 1 < NHG))
                    def _():
                        ws_wait(1 - wslot)
                @pl.when(t + 1 < NS)
                def _():
                    kvs_wait(1 - slot)
                    x_wait(1 - slot)
            return 0
        jax.lax.fori_loop(SS, NS, step, 0)
        with NSC("tail"):
            for b in range(8):
                out_cp(b).wait()

    def fn(A_x, A_k, A_v, A_wq, A_wo, B_x, B_k, B_v, B_wq, B_wo):
        def kvr(a): return jnp.swapaxes(a, 2, 3).reshape(8, 16, 384, 1024)
        anys = pl.BlockSpec(memory_space=pl.ANY)
        V = pltpu.VMEM
        return pl.pallas_call(kernel,
            in_specs=[anys]*10,
            out_specs=anys,
            out_shape=jax.ShapeDtypeStruct((8,240,1280), bf16),
            scratch_shapes=[V((2,2,240,640), bf16), V((2,NP,4,384,1024), bf16),
                  V((2,NP,2,640,384), bf16), V((2,NP,2,384,640), bf16),
                  V((8,240,1280), f32), V((8,240,1280), bf16),
                  pltpu.SemaphoreType.DMA((2,NP)), pltpu.SemaphoreType.DMA((2,)), pltpu.SemaphoreType.DMA((NP,)), pltpu.SemaphoreType.DMA((8,))],
            compiler_params=pltpu.CompilerParams(vmem_limit_bytes=vmem, flags=flags, disable_bounds_checks=nobc),
            name="gqa",
        )(A_x, kvr(A_k), kvr(A_v), A_wq, A_wo, B_x, kvr(B_k), kvr(B_v), B_wq, B_wo)
    return jax.jit(fn)


_kernel_fn = make(NP=4)


@jax.jit
def pallas_concat_heads__gqa_block_cached__gqa_block_cached__near_ridge_kernel(
    A_x, A_k_cache, A_v_cache, A_wq, A_wo, B_x, B_k_cache, B_v_cache, B_wq, B_wo,
):
    return _kernel_fn(A_x, A_k_cache, A_v_cache, A_wq, A_wo, B_x, B_k_cache, B_v_cache, B_wq, B_wo)
```

```python
import re

import jax
import jax.numpy as jnp
import numpy as np
from jax.experimental import pallas as pl
from jax.experimental.pallas import tpu as pltpu

_B, _SQ, _D, _H, _SK, _DH = 8, 240, 640, 32, 1024, 192
_PW = 2 * _DH
_NPAIR = _H // 2
_NP = 4
_NHG = _NPAIR // _NP
_NS = _B * _NHG
_NRAMP = 2 * _NP

_QSCALE = float(_DH ** -0.5 * np.log2(np.e))
_NT = (((1,), (1,)), ((), ()))

_STEP_ORDER = (
    "qp0 qp1 qk0 qk1 pb0 qk2 pa1 qk3 pb2 pa2 pa0 pb3 pb1 pa3 op0 op1 "
    "qp2 qk4 qp3 pb4 qk5 qk6 pb5 pa4 qk7 pb6 pa5 pa7 pb7 pa6 op2 op3 "
    "qp5 qp4 qk8 qk9 pa8 qk10 pb9 pa9 pa10 qk11 pb8 pb10 op4 pa11 pb11 "
    "qp6 qp7 op5 qk12 qk13 pa12 pb12 pa13 qk14 qk15 pb14 pa14 pb13 pb15 pa15 op6 op7"
)
_RAMP_ORDER = "w0 qp0 qk0 qp1 pb0 qk1 pa0 qk2 pb1 pa1 pb2 qk3 pa2 pb3 pa3 op0 op1"
_FIRST_ORDER = ("w0 qp0 w1 qp1 w2 qk0 qk1 w3 pb0 pa0 pb1 pa1 w4 qk2 qk3 w5 "
                "pb2 pa2 pb3 pa3 w6 op0 op1")

_WO_ROWS = ((0, 0, 128), (192, 128, 128), (128, 256, 64), (320, 320, 64))


def _parse(order):
    return [(m.group(1), int(m.group(2))) for m in re.finditer(r"([a-z]+)(\d+)", order)]


def _low_half():
    return jax.lax.broadcasted_iota(jnp.int32, (_SQ, 128), 1) < 64


def _q_proj(x, wq):
    q = jnp.dot(x, wq, preferred_element_type=jnp.float32) * _QSCALE
    q = q.astype(jnp.bfloat16)
    t0, t1, t2 = q[:, 0:128], q[:, 128:256], q[:, 256:384]
    lo, zero = _low_half(), jnp.zeros_like(t1)
    return (jnp.concatenate([t0, jnp.where(lo, t1, zero)], axis=1),
            jnp.concatenate([jnp.where(lo, zero, t1), t2], axis=1))


def _softmax(s):
    m = jnp.max(s, axis=1, keepdims=True)
    p = jnp.exp2(s - m).astype(jnp.bfloat16)
    return p, jnp.sum(p.astype(jnp.float32), axis=1, keepdims=True)


def _reciprocal(l):
    r = pl.reciprocal(l, approx=True)
    return r * (2.0 - l * r)


def _o_proj(head0, head1, wo):
    (oa0, obt0, l0), (oa1, obt1, l1) = head0, head1
    ob = jnp.concatenate([obt0, obt1], axis=0).T
    i0, i1 = _reciprocal(l0), _reciprocal(l1)
    o = jnp.concatenate(
        [oa0 * i0, oa1 * i1, ob * jnp.where(_low_half(), i0, i1)], axis=1)
    return jnp.dot(o.astype(jnp.bfloat16), wo, preferred_element_type=jnp.float32)


def _run(order, x, wq, kv, wo, acc, stage, wait=None, first=False):
    q, s_, p, l, oa, obt = {}, {}, {}, {}, {}, {}
    for op, i in _parse(order):
        if op == "w":
            wait(i)
        elif op == "qp":
            s, j = i % 2, i // 2
            q[2 * i], q[2 * i + 1] = _q_proj(x(s)[...], wq(s, j)[...])
        elif op == "qk":
            s, j, h = (i // 2) % 2, i // 4, i % 2
            kt = kv(s, j)[128 * h:128 * h + 256, :]
            s_[i] = jnp.dot(q.pop(i), kt, preferred_element_type=jnp.float32)
        elif op in ("pa", "pb"):
            s, j, h = (i // 2) % 2, i // 4, i % 2
            if i not in p:
                p[i], l[i] = _softmax(s_.pop(i))
            vt, r = kv(2 + s, j), _DH * h
            if op == "pa":
                oa[i] = jax.lax.dot_general(p[i], vt[r:r + 128, :], _NT,
                                            preferred_element_type=jnp.float32)
            else:
                obt[i] = jax.lax.dot_general(vt[r + 128:r + _DH, :], p[i], _NT,
                                             preferred_element_type=jnp.float32)
        else:
            assert op == "op"
            s, j = i % 2, i // 2
            heads = [(oa.pop(h), obt.pop(h), l.pop(h)) for h in (2 * i, 2 * i + 1)]
            r = _o_proj(heads[0], heads[1], wo(s, j)[...])
            cols = slice(_D * s, _D * s + _D)
            if not first:
                r = acc[:, cols] + r
            acc[:, cols] = r
            stage[:, cols] = r.astype(jnp.bfloat16)


def _kernel(xa_h, ka_h, va_h, wqa_h, woa_h, xb_h, kb_h, vb_h, wqb_h, wob_h, out_h,
            xbuf,
            kv,
            wq,
            wo,
            acc,
            stage,
            s_kv, s_x, s_w, s_out, s_first, s_ramp):
    kv_h, x_h = (ka_h, kb_h, va_h, vb_h), (xa_h, xb_h)
    wq_h, wo_h = (wqa_h, wqb_h), (woa_h, wob_h)
    copy = pltpu.make_async_copy

    def wait_all(ref, sem):
        copy(ref, ref, sem).wait()

    def x_start(s, b, slot, sem):
        copy(x_h[s].at[b], xbuf.at[slot, s], sem).start()

    def kv_pair_start(i, b, pair, slot, j, sem):
        copy(kv_h[i].at[b, pair], kv.at[slot, i, j], sem).start()

    def wq_start(s, pair, wslot, j, sem):
        cols = pl.ds(pl.multiple_of(pair * _PW, _PW), _PW)
        copy(wq_h[s].at[:, cols], wq.at[wslot, j, s], sem).start()

    def wo_start(s, pair, wslot, j, sem):
        for src, dst, n in _WO_ROWS:
            rows = pl.ds(pl.multiple_of(pair * _PW + src, 64), n)
            copy(wo_h[s].at[rows, :], wo.at[wslot, j, s, pl.ds(dst, n), :], sem).start()

    def step_start(t, slot):
        b, hg = t & 7, t >> 3
        for i in range(4):
            copy(kv_h[i].at[b, pl.ds(hg * _NP, _NP)], kv.at[slot, i], s_kv.at[slot, 0]).start()
        for s in range(2):
            x_start(s, b, slot, s_x.at[slot])

    def out_copy(b):
        return copy(stage.at[b], out_h.at[b], s_out.at[b])

    def run(order, slot, wslot, b, pair_slot, **kw):
        _run(order, lambda s: xbuf.at[slot, s], lambda s, j: wq.at[wslot, pair_slot(j), s],
             lambda i, j: kv.at[slot, i, pair_slot(j)],
             lambda s, j: wo.at[wslot, pair_slot(j), s], acc.at[b], stage.at[b], **kw)

    for s in range(2):
        x_start(s, 0, 0, s_first.at[s])
        wq_start(s, 0, 0, 0, s_first.at[s])
    for k, i in enumerate((0, 2, 1, 3)):
        kv_pair_start(i, 0, 0, 0, 0, s_first.at[2 + k])
    for s in range(2):
        wo_start(s, 0, 0, 0, s_first.at[6])
    for s in range(2):
        x_start(s, 1, 1, s_x.at[1])

    def ramp_issue(i, carry):
        b, j, sem = i & 1, i >> 1, s_ramp.at[i]

        @pl.when(b == 0)
        def _():
            for s in range(2):
                wq_start(s, j, 0, j, sem)
        for t in (0, 2, 1, 3):
            kv_pair_start(t, b, j, b, j, sem)

        @pl.when(b == 0)
        def _():
            for s in range(2):
                wo_start(s, j, 0, j, sem)
        return carry

    jax.lax.fori_loop(1, _NRAMP, ramp_issue, 0)
    acc[1:_B] = jnp.zeros((_B - 1, _SQ, 2 * _D), jnp.float32)

    def first_wait(k):
        if k < 2:
            wait_all(xbuf.at[0, k], s_first.at[k])
            wait_all(wq.at[0, 0, k], s_first.at[k])
        elif k < 6:
            wait_all(kv.at[0, (0, 2, 1, 3)[k - 2], 0], s_first.at[k])
        else:
            wait_all(wo.at[0, 0], s_first.at[6])

    run(_FIRST_ORDER, 0, 0, 0, lambda j: 0, wait=first_wait, first=True)

    def ramp_unit(i, carry):
        b, j, sem = i & 1, i >> 1, s_ramp.at[i]

        @pl.when(b == 1)
        def _():
            for t in (0, 2, 1, 3):
                kv_pair_start(t, 2, j, 0, j, s_kv.at[0, j])

        @pl.when(i == _NRAMP - 1)
        def _():
            for s in range(2):
                x_start(s, 2, 0, s_x.at[0])

        def ramp_wait(_):
            @pl.when(i == 1)
            def _():
                wait_all(xbuf.at[1], s_x.at[1])

            @pl.when(b == 0)
            def _():
                wait_all(wq.at[0, j], sem)
                wait_all(wo.at[0, j], sem)
            wait_all(kv.at[b, :, j], sem)

        run(_RAMP_ORDER, b, 0, b, lambda _: j, wait=ramp_wait)
        return carry

    jax.lax.fori_loop(1, _NRAMP, ramp_unit, 0)
    step_start(3, 1)
    for j in range(_NP):
        wait_all(kv.at[0, :, j], s_kv.at[0, j])
    wait_all(xbuf.at[0], s_x.at[0])

    def step(t, carry):
        b, hg, slot = t & 7, t >> 3, t & 1
        wslot = hg & 1
        run(_STEP_ORDER, slot, wslot, b, lambda j: j)

        @pl.when(t + 2 < _NS)
        def _():
            step_start(t + 2, slot)

        @pl.when(hg == _NHG - 1)
        def _():
            out_copy(b).start()

        @pl.when(jnp.logical_and(b == 4, hg + 1 < _NHG))
        def _():
            for j in range(_NP):
                for s in range(2):
                    wq_start(s, (hg + 1) * _NP + j, 1 - wslot, j, s_w.at[0])
                for s in range(2):
                    wo_start(s, (hg + 1) * _NP + j, 1 - wslot, j, s_w.at[0])

        @pl.when(jnp.logical_and(b == 7, hg + 1 < _NHG))
        def _():
            wait_all(wq.at[1 - wslot], s_w.at[0])
            wait_all(wo.at[1 - wslot], s_w.at[0])

        @pl.when(t + 1 < _NS)
        def _():
            wait_all(kv.at[1 - slot], s_kv.at[1 - slot, 0])
            wait_all(xbuf.at[1 - slot], s_x.at[1 - slot])
        return carry

    jax.lax.fori_loop(2, _NS, step, 0)
    for b in range(_B):
        out_copy(b).wait()


@jax.jit
def pallas_concat_heads__gqa_block_cached__gqa_block_cached__near_ridge_kernel(
    A_x: jax.Array,
    A_k_cache: jax.Array,
    A_v_cache: jax.Array,
    A_wq: jax.Array,
    A_wo: jax.Array,
    B_x: jax.Array,
    B_k_cache: jax.Array,
    B_v_cache: jax.Array,
    B_wq: jax.Array,
    B_wo: jax.Array,
):
    def pairs(a):
        return jnp.swapaxes(a, 2, 3).reshape(_B, _NPAIR, _PW, _SK)

    bf16, f32 = jnp.bfloat16, jnp.float32
    vmem, dma = pltpu.VMEM, pltpu.SemaphoreType.DMA
    hbm = pl.BlockSpec(memory_space=pl.ANY)
    return pl.pallas_call(
        _kernel,
        in_specs=[hbm] * 10,
        out_specs=hbm,
        out_shape=jax.ShapeDtypeStruct((_B, _SQ, 2 * _D), bf16),
        scratch_shapes=[
            vmem((2, 2, _SQ, _D), bf16),
            vmem((2, 4, _NP, _PW, _SK), bf16),
            vmem((2, _NP, 2, _D, _PW), bf16),
            vmem((2, _NP, 2, _PW, _D), bf16),
            vmem((_B, _SQ, 2 * _D), f32),
            vmem((_B, _SQ, 2 * _D), bf16),
            dma((2, _NP)), dma((2,)), dma((1,)), dma((_B,)), dma((7,)), dma((_NRAMP,)),
        ],
        compiler_params=pltpu.CompilerParams(
            vmem_limit_bytes=110 * 1024 * 1024,
            disable_bounds_checks=True,
        ),
        name="gqa2_cached",
    )(A_x, pairs(A_k_cache), pairs(A_v_cache), A_wq, A_wo,
      B_x, pairs(B_k_cache), pairs(B_v_cache), B_wq, B_wo)
```

```python
import re

import jax
import jax.numpy as jnp
import numpy as np
from jax.experimental import pallas as pl
from jax.experimental.pallas import tpu as pltpu

_B, _SQ, _D, _H, _SK, _DH = 8, 240, 640, 32, 1024, 192
_PW = 2 * _DH
_NPAIR = _H // 2
_NP = 4
_NHG = _NPAIR // _NP
_NS = _B * _NHG
_NRAMP = 2 * _NP

_QSCALE = float(_DH ** -0.5 * np.log2(np.e))
_NT = (((1,), (1,)), ((), ()))

_STEP_ORDER = (
    "qp0 qp1 qk0 qk1 pb0 qk2 pa1 qk3 pb2 pa2 pa0 pb3 pb1 pa3 op0 op1 "
    "qp2 qk4 qp3 pb4 qk5 qk6 pb5 pa4 qk7 pb6 pa5 pa7 pa6 pb7 op2 op3 "
    "qp5 qp4 qk8 qk9 pa8 qk10 pb9 pa9 pa10 qk11 pb8 pb10 op4 pa11 pb11 qp6 "
    "qp7 op5 qk12 qk13 pa12 pb12 pa13 qk14 qk15 pb14 pa14 pb13 pb15 pa15 op6 op7"
)
_RAMP_ORDER = "w0 qp0 qk0 qp1 pb0 qk1 pa0 qk2 pb1 pa1 pb2 qk3 pa2 pb3 pa3 op0 op1"
_FIRST_ORDER = ("w0 qp0 w1 qp1 w2 qk0 qk1 w3 pb0 pa0 pb1 pa1 w4 qk2 qk3 w5 "
                "pb2 pa2 pb3 pa3 w6 op0 op1")

_WO_ROWS = ((0, 0, 128), (192, 128, 128), (128, 256, 64), (320, 320, 64))


def _parse(order):
    return [(m.group(1), int(m.group(2))) for m in re.finditer(r"([a-z]+)(\d+)", order)]


def _low_half():
    return jax.lax.broadcasted_iota(jnp.int32, (_SQ, 128), 1) < 64


def _q_proj(x, wq):
    q = jnp.dot(x, wq, preferred_element_type=jnp.float32) * _QSCALE
    q = q.astype(jnp.bfloat16)
    t0, t1, t2 = q[:, 0:128], q[:, 128:256], q[:, 256:384]
    lo, zero = _low_half(), jnp.zeros_like(t1)
    return (jnp.concatenate([t0, jnp.where(lo, t1, zero)], axis=1),
            jnp.concatenate([jnp.where(lo, zero, t1), t2], axis=1))


def _softmax(s):
    m = jnp.max(s, axis=1, keepdims=True)
    p = jnp.exp2(s - m).astype(jnp.bfloat16)
    return p, jnp.sum(p.astype(jnp.float32), axis=1, keepdims=True)


def _reciprocal(l):
    r = pl.reciprocal(l, approx=True)
    return r * (2.0 - l * r)


def _o_proj(head0, head1, wo):
    (oa0, obt0, l0), (oa1, obt1, l1) = head0, head1
    ob = jnp.concatenate([obt0, obt1], axis=0).T
    i0, i1 = _reciprocal(l0), _reciprocal(l1)
    o = jnp.concatenate(
        [oa0 * i0, oa1 * i1, ob * jnp.where(_low_half(), i0, i1)], axis=1)
    return jnp.dot(o.astype(jnp.bfloat16), wo, preferred_element_type=jnp.float32)


def _run(order, x, wq, kv, wo, acc, stage, wait=None, first=False):
    q, s_, p, l, oa, obt = {}, {}, {}, {}, {}, {}
    for op, i in _parse(order):
        if op == "w":
            wait(i)
        elif op == "qp":
            s, j = i % 2, i // 2
            q[2 * i], q[2 * i + 1] = _q_proj(x(s)[...], wq(s, j)[...])
        elif op == "qk":
            s, j, h = (i // 2) % 2, i // 4, i % 2
            kt = kv(s, j)[128 * h:128 * h + 256, :]
            s_[i] = jnp.dot(q.pop(i), kt, preferred_element_type=jnp.float32)
        elif op in ("pa", "pb"):
            s, j, h = (i // 2) % 2, i // 4, i % 2
            if i not in p:
                p[i], l[i] = _softmax(s_.pop(i))
            vt, r = kv(2 + s, j), _DH * h
            if op == "pa":
                oa[i] = jax.lax.dot_general(p[i], vt[r:r + 128, :], _NT,
                                            preferred_element_type=jnp.float32)
            else:
                obt[i] = jax.lax.dot_general(vt[r + 128:r + _DH, :], p[i], _NT,
                                             preferred_element_type=jnp.float32)
        else:
            assert op == "op"
            s, j = i % 2, i // 2
            heads = [(oa.pop(h), obt.pop(h), l.pop(h)) for h in (2 * i, 2 * i + 1)]
            r = _o_proj(heads[0], heads[1], wo(s, j)[...])
            cols = slice(_D * s, _D * s + _D)
            if not first:
                r = acc[:, cols] + r
            acc[:, cols] = r
            stage[:, cols] = r.astype(jnp.bfloat16)


def _kernel(xa_h, ka_h, va_h, wqa_h, woa_h, xb_h, kb_h, vb_h, wqb_h, wob_h, out_h,
            xbuf,
            kv,
            wq,
            wo,
            acc,
            stage,
            s_kv, s_x, s_w, s_out, s_first, s_ramp):
    kv_h, x_h = (ka_h, kb_h, va_h, vb_h), (xa_h, xb_h)
    wq_h, wo_h = (wqa_h, wqb_h), (woa_h, wob_h)
    copy = pltpu.make_async_copy

    def wait_all(ref, sem):
        copy(ref, ref, sem).wait()

    def x_start(s, b, slot, sem):
        copy(x_h[s].at[b], xbuf.at[slot, s], sem).start()

    def kv_pair_start(i, b, pair, slot, j, sem):
        copy(kv_h[i].at[b, pair], kv.at[slot, i, j], sem).start()

    def wq_start(s, pair, wslot, j, sem):
        cols = pl.ds(pl.multiple_of(pair * _PW, _PW), _PW)
        copy(wq_h[s].at[:, cols], wq.at[wslot, j, s], sem).start()

    def wo_start(s, pair, wslot, j, sem):
        for src, dst, n in _WO_ROWS:
            rows = pl.ds(pl.multiple_of(pair * _PW + src, 64), n)
            copy(wo_h[s].at[rows, :], wo.at[wslot, j, s, pl.ds(dst, n), :], sem).start()

    def step_start(t, slot):
        b, hg = t & 7, t >> 3
        for i in range(4):
            copy(kv_h[i].at[b, pl.ds(hg * _NP, _NP)], kv.at[slot, i], s_kv.at[slot, 0]).start()
        for s in range(2):
            x_start(s, b, slot, s_x.at[slot])

    def out_copy(b):
        return copy(stage.at[b], out_h.at[b], s_out.at[b])

    def run(order, slot, wslot, b, pair_slot, **kw):
        _run(order, lambda s: xbuf.at[slot, s], lambda s, j: wq.at[wslot, pair_slot(j), s],
             lambda i, j: kv.at[slot, i, pair_slot(j)],
             lambda s, j: wo.at[wslot, pair_slot(j), s], acc.at[b], stage.at[b], **kw)

    for s in range(2):
        x_start(s, 0, 0, s_first.at[2 * s])
        wq_start(s, 0, 0, 0, s_first.at[2 * s + 1])
    for k, i in enumerate((0, 2, 1, 3)):
        kv_pair_start(i, 0, 0, 0, 0, s_first.at[4 + k])
    for s in range(2):
        wo_start(s, 0, 0, 0, s_first.at[8])
    for s in range(2):
        x_start(s, 1, 1, s_x.at[1])

    def ramp_issue(i, carry):
        b, j = i & 1, i >> 1

        @pl.when(b == 0)
        def _():
            for s in range(2):
                wq_start(s, j, 0, j, s_ramp.at[i, 0])
        for t in (0, 2, 1, 3):
            kv_pair_start(t, b, j, b, j, s_ramp.at[i, 2])

        @pl.when(b == 0)
        def _():
            for s in range(2):
                wo_start(s, j, 0, j, s_ramp.at[i, 1])
        return carry

    jax.lax.fori_loop(1, _NRAMP, ramp_issue, 0)
    acc[1:_B] = jnp.zeros((_B - 1, _SQ, 2 * _D), jnp.float32)

    def first_wait(k):
        if k < 2:
            wait_all(xbuf.at[0, k], s_first.at[2 * k])
            wait_all(wq.at[0, 0, k], s_first.at[2 * k + 1])
        elif k < 6:
            wait_all(kv.at[0, (0, 2, 1, 3)[k - 2], 0], s_first.at[k + 2])
        else:
            wait_all(wo.at[0, 0], s_first.at[8])

    run(_FIRST_ORDER, 0, 0, 0, lambda j: 0, wait=first_wait, first=True)

    def ramp_unit(i, carry):
        b, j = i & 1, i >> 1

        @pl.when(b == 1)
        def _():
            for t in (0, 2, 1, 3):
                kv_pair_start(t, 2, j, 0, j, s_kv.at[0, j])

        @pl.when(i == _NRAMP - 1)
        def _():
            for s in range(2):
                x_start(s, 2, 0, s_x.at[0])

        def ramp_wait(_):
            @pl.when(i == 1)
            def _():
                wait_all(xbuf.at[1], s_x.at[1])

            @pl.when(b == 0)
            def _():
                wait_all(wq.at[0, j], s_ramp.at[i, 0])
                wait_all(wo.at[0, j], s_ramp.at[i, 1])
            wait_all(kv.at[b, :, j], s_ramp.at[i, 2])

        run(_RAMP_ORDER, b, 0, b, lambda _: j, wait=ramp_wait)
        return carry

    jax.lax.fori_loop(1, _NRAMP, ramp_unit, 0)
    step_start(3, 1)
    for j in range(_NP):
        wait_all(kv.at[0, :, j], s_kv.at[0, j])
    wait_all(xbuf.at[0], s_x.at[0])

    def step(t, carry):
        b, hg, slot = t & 7, t >> 3, t & 1
        wslot = hg & 1
        run(_STEP_ORDER, slot, wslot, b, lambda j: j)

        @pl.when(t + 2 < _NS)
        def _():
            step_start(t + 2, slot)

        @pl.when(hg == _NHG - 1)
        def _():
            out_copy(b).start()

        @pl.when(jnp.logical_and(b == 4, hg + 1 < _NHG))
        def _():
            for j in range(_NP):
                for s in range(2):
                    wq_start(s, (hg + 1) * _NP + j, 1 - wslot, j, s_w.at[0])
                for s in range(2):
                    wo_start(s, (hg + 1) * _NP + j, 1 - wslot, j, s_w.at[1])

        @pl.when(jnp.logical_and(b == 7, hg + 1 < _NHG))
        def _():
            wait_all(wq.at[1 - wslot], s_w.at[0])
            wait_all(wo.at[1 - wslot], s_w.at[1])

        @pl.when(t + 1 < _NS)
        def _():
            wait_all(kv.at[1 - slot], s_kv.at[1 - slot, 0])
            wait_all(xbuf.at[1 - slot], s_x.at[1 - slot])
        return carry

    jax.lax.fori_loop(2, _NS, step, 0)
    for b in range(_B):
        out_copy(b).wait()


@jax.jit
def pallas_concat_heads__gqa_block_cached__gqa_block_cached__near_ridge_kernel(
    A_x: jax.Array,
    A_k_cache: jax.Array,
    A_v_cache: jax.Array,
    A_wq: jax.Array,
    A_wo: jax.Array,
    B_x: jax.Array,
    B_k_cache: jax.Array,
    B_v_cache: jax.Array,
    B_wq: jax.Array,
    B_wo: jax.Array,
):
    def pairs(a):
        return jnp.swapaxes(a, 2, 3).reshape(_B, _NPAIR, _PW, _SK)

    bf16, f32 = jnp.bfloat16, jnp.float32
    vmem, dma = pltpu.VMEM, pltpu.SemaphoreType.DMA
    hbm = pl.BlockSpec(memory_space=pl.ANY)
    return pl.pallas_call(
        _kernel,
        in_specs=[hbm] * 10,
        out_specs=hbm,
        out_shape=jax.ShapeDtypeStruct((_B, _SQ, 2 * _D), bf16),
        scratch_shapes=[
            vmem((2, 2, _SQ, _D), bf16),
            vmem((2, 4, _NP, _PW, _SK), bf16),
            vmem((2, _NP, 2, _D, _PW), bf16),
            vmem((2, _NP, 2, _PW, _D), bf16),
            vmem((_B, _SQ, 2 * _D), f32),
            vmem((_B, _SQ, 2 * _D), bf16),
            dma((2, _NP)), dma((2,)), dma((2,)), dma((_B,)), dma((9,)), dma((_NRAMP, 3)),
        ],
        compiler_params=pltpu.CompilerParams(
            vmem_limit_bytes=110 * 1024 * 1024,
            disable_bounds_checks=True,
        ),
        name="gqa2_cached",
    )(A_x, pairs(A_k_cache), pairs(A_v_cache), A_wq, A_wo,
      B_x, pairs(B_k_cache), pairs(B_v_cache), B_wq, B_wo)
```
